```python
import os as _os
_os.environ.setdefault("JAX_PLATFORMS", "cpu")
import jax
import jax.numpy as jnp

def _softmax(x, axis=-1):
    return jax.nn.softmax(x, axis=axis)
def _gelu(x):
    return jax.nn.gelu(x, approximate=True)
def _silu(x):
    return jax.nn.silu(x)
def _sigmoid(x):
    return jax.nn.sigmoid(x)
def _layernorm(x, axis=-1, eps=1e-5):
    m = jnp.mean(x, axis=axis, keepdims=True)
    v = jnp.var(x, axis=axis, keepdims=True)
    return (x - m) / jnp.sqrt(v + eps)
def _scatter_add(tgt, idx, src, axis=0):
    return tgt.at[idx].add(src)
def _segment_sum(src, seg, n):
    return jax.ops.segment_sum(src, seg, n)
class _Rng:
    def __init__(self, key):
        self._k = key
    def _next(self):
        self._k, sub = jax.random.split(self._k)
        return sub
    def normal(self, shape):
        return jax.random.normal(self._next(), shape, dtype=jnp.bfloat16)
    def randint(self, lo, hi, shape):
        return jax.random.randint(self._next(), shape, lo, hi, dtype=jnp.int32)
    def uniform(self, shape, lo=0.0, hi=1.0):
        return jax.random.uniform(self._next(), shape, jnp.bfloat16, lo, hi)
    def permutation(self, n):
        return jax.random.permutation(self._next(), n)


kernel_name = 'gated_mix__mha_block__mixer_s_mlp__prompt'

def setup_inputs():
    _rng = _Rng(jax.random.key(int.from_bytes(__import__("os").urandom(4), "little")))
    _w = (lambda a: (lambda t: t.astype(jnp.bfloat16) if jnp.issubdtype(t.dtype, jnp.floating) else t)(jnp.asarray(a)))
    def _A_setup():
        B, S, D, H = 1, 2048, 512, 32
        return {
            "x": _w((lambda *s: _rng.normal(s) * 0.05)(B, S, D)),
            "wqkv": _w((lambda *s: _rng.normal(s) * 0.8)(D, 3 * D)),
            "wo": _w((lambda *s: _rng.normal(s) * 0.05)(D, D)),
        }
    _A_in = _A_setup()

    def _B_setup():
        B, S, D, F = 1, 2048, 512, 1792
        return {
            "x":  _w((lambda *s: _rng.normal(s) * 0.05)(B, S, D)),
            "w1": _w((lambda *s: _rng.normal(s) * 0.2)(D, D) * (D ** -0.5)),
            "w2": _w((lambda *s: _rng.normal(s) * 0.2)(D, D) * (D ** -0.5)),
            "w3": _w((lambda *s: _rng.normal(s) * 0.2)(D, F) * (D ** -0.5)),
            "w4": _w((lambda *s: _rng.normal(s) * 0.2)(F, D) * (F ** -0.5)),
        }
    _B_in = _B_setup()

    return {
        "A_x": _A_in["x"],
        "A_wqkv": _A_in["wqkv"],
        "A_wo": _A_in["wo"],
        "B_x": _B_in["x"],
        "B_w1": _B_in["w1"],
        "B_w2": _B_in["w2"],
        "B_w3": _B_in["w3"],
        "B_w4": _B_in["w4"],
        "gate_w": _w((lambda *s: _rng.normal(s) * 0.05)(512) * 16.0),
    }

def reference(A_x, A_wqkv, A_wo, B_x, B_w1, B_w2, B_w3, B_w4, gate_w):
    def _A_ref(x, wqkv, wo):
        B, S, D = x.shape
        H = 32
        Dh = D // H
        qkv = (lambda x, *d: x.transpose(*d))((x @ wqkv).reshape(B, S, 3, H, Dh), 2, 0, 3, 1, 4)
        q, k, v = qkv[0], qkv[1], qkv[2]
        scores = jnp.einsum("bhqd,bhkd->bhqk", q, k) * (Dh ** -0.5)
        p = _softmax(scores, axis=-1)
        o = jnp.einsum("bhqk,bhkd->bhqd", p, v)
        return (lambda x, *d: x.transpose(*d))(o, 0, 2, 1, 3).reshape(B, S, D) @ wo

    def _B_ref(x, w1, w2, w3, w4):
        B, S, D = x.shape
        h = _gelu(_layernorm(x, axis=-1) @ w1)
        c = D // 4
        g0 = jnp.pad(h[:, :, 0*c:1*c], ((0, 0), (1, 0), (0, 0)))[:, :S, :]
        g1 = jnp.pad(h[:, :, 1*c:2*c], ((0, 0), (0, 1), (0, 0)))[:, 1:, :]
        g2 = jnp.pad(h[:, :, 2*c:3*c], ((0, 0), (2, 0), (0, 0)))[:, :S, :]
        g3 = jnp.pad(h[:, :, 3*c:   ], ((0, 0), (0, 2), (0, 0)))[:, 2:, :]
        hs = jnp.concatenate([g0, g1, g2, g3], axis=-1) @ w2
        x1 = x + hs
        h2 = _gelu(_layernorm(x1, axis=-1) @ w3) @ w4
        return x1 + h2

    x = A_x
    g = _sigmoid((x * gate_w).sum(-1, keepdims=True))
    a = _A_ref(x, A_wqkv, A_wo)
    b = _B_ref(x, B_w1, B_w2, B_w3, B_w4)
    return g * a + (1 - g) * b
```

```python
import jax
import jax.numpy as jnp
import jax.experimental.pallas as pl
import jax.experimental.pallas.tpu as pltpu

S = 2048
D = 512
H = 32
DH = 16
F = 1792
TQ = 512
KC = 128
NC = S // KC
LA = 3
HPI = 4
NSLOT = 16
XC = 4
XR = S // XC
PAD = 8
LOG2E = 1.4426950408889634
EPS = 1e-5

_NT = (((1,), (1,)), ((), ()))
_TN = (((0,), (0,)), ((), ()))
_bf = jnp.bfloat16
_f32 = jnp.float32


def _gelu(x):
    c = 0.7978845608028654
    return 0.5 * x * (1.0 + jnp.tanh(c * (x + 0.044715 * (x * x * x))))


def _pack(x):
    return pltpu.bitcast(x, jnp.uint32)


def _unpack(x):
    return pltpu.bitcast(x, _bf)


def _layernorm(x):
    m = jnp.mean(x, axis=-1, keepdims=True)
    xc = x - m
    v = jnp.mean(xc * xc, axis=-1, keepdims=True)
    return xc * jax.lax.rsqrt(v + EPS)


def _kernel(x_hbm, wqkv_hbm, wo_hbm, w1_hbm, w2_hbm, w3_hbm, w4_hbm, gw_ref,
            o_ref,
            x_v, wq_v, wk_v, wv_v, wo_v, w1_v, w2_v, w3_v, w4_v, sems,
            k_scr, qt_scr, vt_scr, m_scr, h_scr, acc_scr, l_scr, p_scr, gb_scr):
    i = pl.program_id(0)

    def x_copy(c):
        return pltpu.make_async_copy(x_hbm.at[pl.ds(c * XR, XR), :], x_v.at[pl.ds(c * XR, XR), :],
                                     sems.at[c])

    def wqkv_copy(part):
        dst = [wq_v, wk_v, wv_v][part]
        return pltpu.make_async_copy(wqkv_hbm.at[:, pl.ds(part * D, D)], dst, sems.at[XC + part])

    def w_copy(j):
        src, dst = [(w1_hbm, w1_v), (wo_hbm, wo_v), (w2_hbm, w2_v), (w3_hbm, w3_v), (w4_hbm, w4_v)][j]
        return pltpu.make_async_copy(src, dst, sems.at[XC + 3 + j])

    @pl.when(i == 0)
    def _prologue():
        wqkv_copy(1).start()
        x_copy(0).start()
        x_copy(1).start()
        w_copy(0).start()
        wqkv_copy(0).start()
        wqkv_copy(2).start()
        x_copy(2).start()
        x_copy(3).start()
        for j in range(1, 5):
            w_copy(j).start()

        grp = (jax.lax.broadcasted_iota(jnp.int32, (H, D), 1) // DH
               == jax.lax.broadcasted_iota(jnp.int32, (H, D), 0)).astype(_bf)

        def k_proj(c):
            kb = jnp.dot(x_v[c * XR:(c + 1) * XR, :], wk_v[...],
                         preferred_element_type=_f32).astype(_bf)
            k_scr[c * XR // 2:(c + 1) * XR // 2, :] = _pack(kb)
            kf = kb.astype(_f32)
            return (kf * kf).astype(_bf)

        def k_norm2(k2):
            n2 = jax.lax.dot_general(grp, k2, _NT, preferred_element_type=_f32)
            return jnp.max(n2.reshape(H, XR // 128, 128), axis=1)

        def ln_x(c):
            return _layernorm(x_v[c * XR:(c + 1) * XR, :].astype(_f32)).astype(_bf)

        def h_proj(c, ln):
            hh = _gelu(jnp.dot(ln, w1_v[...], preferred_element_type=_f32))
            h_scr[PAD + c * XR:PAD + (c + 1) * XR, :] = hh.astype(_bf).astype(_f32)

        h_scr[0:PAD, :] = jnp.zeros((PAD, D), _f32)
        h_scr[PAD + S:PAD + S + PAD, :] = jnp.zeros((PAD, D), _f32)
        for sl in range(NSLOT - LA, NSLOT):
            p_scr[sl] = jnp.zeros((KC, TQ), _bf)

        wqkv_copy(1).wait()
        x_copy(0).wait()
        k2_0 = k_proj(0)
        ln_0 = ln_x(0)
        x_copy(1).wait()
        k2_1 = k_proj(1)
        ln_1 = ln_x(1)
        w_copy(0).wait()
        h_proj(0, ln_0)
        kn2 = k_norm2(k2_0)
        h_proj(1, ln_1)
        kn2 = jnp.maximum(kn2, k_norm2(k2_1))
        wqkv_copy(0).wait()
        wqkv_copy(2).wait()
        x_copy(2).wait()
        x_copy(3).wait()
        wq_t = wq_v[...].astype(_f32).T.astype(_bf)
        wv_t = wv_v[...].astype(_f32).T.astype(_bf)
        k2_2 = k_proj(2)
        ln_2 = ln_x(2)
        k2_3 = k_proj(3)
        ln_3 = ln_x(3)
        h_proj(2, ln_2)
        kn2 = jnp.maximum(kn2, k_norm2(k2_2))
        h_proj(3, ln_3)
        kn2 = jnp.maximum(kn2, k_norm2(k2_3))
        kn2 = jnp.max(kn2, axis=1, keepdims=True)
        xa = x_v[...]
        qt = jax.lax.dot_general(wq_t, xa, _NT, preferred_element_type=_f32)
        qtb = (qt * (DH ** -0.5 * LOG2E)).astype(_bf)
        qt_scr[...] = qtb
        vt_scr[...] = _pack(
            jax.lax.dot_general(wv_t, xa, _NT, preferred_element_type=_f32).astype(_bf))
        qf = qtb.astype(_f32)
        qn2 = jnp.sum((qf * qf).reshape(H, DH, S), axis=1)
        m_scr[...] = jnp.sqrt(qn2 * kn2) * 1.02
        for j in range(1, 5):
            w_copy(j).wait()

    q0 = pl.multiple_of(i * TQ, TQ)
    rows = jax.lax.broadcasted_iota(jnp.int32, (128, TQ), 0) // DH

    def masked_q(h):
        goff = pl.multiple_of((h // 8) * 128, 128)
        qg = qt_scr[pl.ds(goff, 128), pl.ds(q0, TQ)]
        return jnp.where(rows == (h % 8), qg, jnp.zeros_like(qg)), goff

    def pv_dot(h, kc, sl):
        vt = _unpack(vt_scr[pl.ds(pl.multiple_of(h * (DH // 2), DH // 2), DH // 2),
                            kc * KC:(kc + 1) * KC])
        return jnp.dot(vt, p_scr[sl], preferred_element_type=_f32)

    def store_acc(h, acc):
        acc_scr[pl.ds(pl.multiple_of((h + 1) * DH, DH), DH), :] = acc

    NW = HPI * NC
    tail = [(NC - LA + t, (NW - LA + t) % NSLOT) for t in range(LA)]

    def fast_heads(g, acc_prev):
        h0 = g * HPI
        qms = [masked_q(h0 + u)[0] for u in range(HPI)]
        goff = masked_q(h0)[1]
        ms = [m_scr[pl.ds(h0 + u, 1), pl.ds(q0, TQ)] for u in range(HPI)]
        work = [(u, kc) for u in range(HPI) for kc in range(NC)]
        accs = [jnp.zeros((DH, TQ), _f32) for _ in range(HPI)]
        ls = [jnp.zeros((8, TQ), _f32) for _ in range(HPI)]

        hprev = jnp.maximum(h0 - 1, 0)
        for kc, sl in tail:
            acc_prev = acc_prev + pv_dot(hprev, kc, sl)
        store_acc(h0 - 1, acc_prev)

        def qk_step(idx):
            u, kc = work[idx]
            kc_val = _unpack(k_scr[kc * KC // 2:(kc + 1) * KC // 2, pl.ds(goff, 128)])
            s = jnp.dot(kc_val, qms[u], preferred_element_type=_f32)
            p32 = jnp.exp2(s - ms[u])
            ls[u] = ls[u] + jnp.sum(p32.reshape(KC // 8, 8, TQ), axis=0)
            p_scr[idx % NSLOT] = p32.astype(_bf)
            if kc == NC - 1:
                l_scr[h0 + u] = ls[u]

        def pv_step(idx):
            u, kc = work[idx]
            accs[u] = accs[u] + pv_dot(h0 + u, kc, idx % NSLOT)
            if kc == NC - 1:
                store_acc(h0 + u, accs[u])

        for idx in range(NW - LA):
            qk_step(idx)
            if idx >= LA:
                pv_step(idx - LA)
        for idx in range(NW - LA, NW):
            qk_step(idx)
        for idx in range(NW - 2 * LA, NW - LA):
            pv_step(idx)
        return accs[HPI - 1]

    acc_last = jax.lax.fori_loop(0, H // HPI, fast_heads, jnp.zeros((DH, TQ), _f32))
    for kc, sl in tail:
        acc_last = acc_last + pv_dot(H - 1, kc, sl)
    store_acc(H - 1, acc_last)

    c = D // 4
    win = h_scr[pl.ds(q0, TQ + 2 * PAD), :]
    hs_in = jnp.concatenate([
        win[PAD - 1:PAD - 1 + TQ, 0 * c:1 * c],
        win[PAD + 1:PAD + 1 + TQ, 1 * c:2 * c],
        win[PAD - 2:PAD - 2 + TQ, 2 * c:3 * c],
        win[PAD + 2:PAD + 2 + TQ, 3 * c:4 * c]], axis=-1).astype(_bf)
    xa_t = x_v[pl.ds(q0, TQ), :].astype(_f32)
    x1 = xa_t + jnp.dot(hs_in, w2_v[...], preferred_element_type=_f32)

    def attn_out():
        l_all = jnp.sum(l_scr[...], axis=1)
        ot = acc_scr[DH:, :].reshape(H, DH, TQ) * (1.0 / l_all)[:, None, :]
        ot = ot.reshape(D, TQ).astype(_bf)
        return jax.lax.dot_general(ot, wo_v[...], _TN, preferred_element_type=_f32), l_all

    a, l_all = attn_out()
    safe = jnp.logical_and(jnp.min(l_all) >= 2.0 ** -79, jnp.max(l_all) <= 2.0 ** 100)

    h3 = _gelu(jnp.dot(_layernorm(x1).astype(_bf), w3_v[...], preferred_element_type=_f32))
    b = x1 + jnp.dot(h3.astype(_bf), w4_v[...], preferred_element_type=_f32)
    g = jax.nn.sigmoid(jnp.sum(xa_t * gw_ref[...].astype(_f32), axis=-1, keepdims=True))
    gb = (1.0 - g) * b
    gb_scr[...] = gb
    o_ref[...] = (g * a + gb).astype(o_ref.dtype)

    @pl.when(jnp.logical_not(safe))
    def _fallback():
        def slow_head(h, carry):
            qm, goff = masked_q(h)
            s = jnp.dot(_unpack(k_scr[:, pl.ds(goff, 128)]), qm, preferred_element_type=_f32)
            p32 = jnp.exp2(s - jnp.max(s, axis=0, keepdims=True))
            l_scr[h] = jnp.sum(p32.reshape(S // 8, 8, TQ), axis=0)
            vt = _unpack(vt_scr[pl.ds(pl.multiple_of(h * (DH // 2), DH // 2), DH // 2), :])
            store_acc(h, jnp.dot(vt, p32.astype(_bf), preferred_element_type=_f32))
            return carry
        jax.lax.fori_loop(0, H, slow_head, 0)
        a2, _ = attn_out()
        g2 = jax.nn.sigmoid(jnp.sum(x_v[pl.ds(q0, TQ), :].astype(_f32) * gw_ref[...].astype(_f32),
                                    axis=-1, keepdims=True))
        o_ref[...] = (g2 * a2 + gb_scr[...]).astype(o_ref.dtype)


@jax.jit
def pallas_gated_mix__mha_block__mixer_s_mlp__prompt_kernel(
    A_x: jax.Array,
    A_wqkv: jax.Array,
    A_wo: jax.Array,
    B_x: jax.Array,
    B_w1: jax.Array,
    B_w2: jax.Array,
    B_w3: jax.Array,
    B_w4: jax.Array,
    gate_w: jax.Array,
):
    hbm = pl.BlockSpec(memory_space=pl.ANY)
    out = pl.pallas_call(
        _kernel,
        grid=(S // TQ,),
        in_specs=[hbm] * 7 + [pl.BlockSpec((1, D), lambda i: (0, 0))],
        out_specs=pl.BlockSpec((TQ, D), lambda i: (i, 0)),
        out_shape=jax.ShapeDtypeStruct((S, D), jnp.bfloat16),
        scratch_shapes=[
            pltpu.VMEM((S, D), _bf),
            pltpu.VMEM((D, D), _bf),
            pltpu.VMEM((D, D), _bf),
            pltpu.VMEM((D, D), _bf),
            pltpu.VMEM((D, D), _bf),
            pltpu.VMEM((D, D), _bf),
            pltpu.VMEM((D, D), _bf),
            pltpu.VMEM((D, F), _bf),
            pltpu.VMEM((F, D), _bf),
            pltpu.SemaphoreType.DMA((XC + 3 + 5,)),
            pltpu.VMEM((S // 2, D), jnp.uint32),
            pltpu.VMEM((D, S), _bf),
            pltpu.VMEM((D // 2, S), jnp.uint32),
            pltpu.VMEM((H, S), _f32),
            pltpu.VMEM((S + 2 * PAD, D), _f32),
            pltpu.VMEM(((H + 1) * DH, TQ), _f32),
            pltpu.VMEM((H, 8, TQ), _f32),
            pltpu.VMEM((NSLOT, KC, TQ), _bf),
            pltpu.VMEM((TQ, D), _f32),
        ],
        compiler_params=pltpu.CompilerParams(
            dimension_semantics=("arbitrary",),
            vmem_limit_bytes=100 * 1024 * 1024),
        name="gated_mix",
    )(A_x.reshape(S, D), A_wqkv, A_wo, B_w1, B_w2, B_w3, B_w4, gate_w.reshape(1, D))
    return out.reshape(1, S, D)
```

```python
import jax
import jax.numpy as jnp
import jax.experimental.pallas as pl
import jax.experimental.pallas.tpu as pltpu

S = 2048
D = 512
H = 32
DH = 16
F = 1792
TQ = 512
KC = 128
NC = S // KC
LA = 3
HPI = 4
NSLOT = 16
XC = 4
XR = S // XC
PAD = 8
LOG2E = 1.4426950408889634
EPS = 1e-5

_NT = (((1,), (1,)), ((), ()))
_TN = (((0,), (0,)), ((), ()))
_bf = jnp.bfloat16
_f32 = jnp.float32


def _gelu(x):
    c = 0.7978845608028654
    return 0.5 * x * (1.0 + jnp.tanh(c * (x + 0.044715 * (x * x * x))))


def _pack(x):
    return pltpu.bitcast(x, jnp.uint32)


def _unpack(x):
    return pltpu.bitcast(x, _bf)


def _layernorm(x):
    m = jnp.mean(x, axis=-1, keepdims=True)
    xc = x - m
    v = jnp.mean(xc * xc, axis=-1, keepdims=True)
    return xc * jax.lax.rsqrt(v + EPS)


def _kernel(x_hbm, wqkv_hbm, wo_hbm, w1_hbm, w2_hbm, w3_hbm, w4_hbm, gw_ref,
            o_ref,
            x_v, wq_v, wk_v, wv_v, wo_v, w1_v, w2_v, w3_v, w4_v, sems,
            k_scr, qt_scr, vt_scr, m_scr, h_scr, acc_scr, l_scr, p_scr, gb_scr):
    i = pl.program_id(0)

    def x_copy(c):
        return pltpu.make_async_copy(x_hbm.at[pl.ds(c * XR, XR), :], x_v.at[pl.ds(c * XR, XR), :],
                                     sems.at[c])

    def wqkv_copy(part):
        dst = [wq_v, wk_v, wv_v][part]
        return pltpu.make_async_copy(wqkv_hbm.at[:, pl.ds(part * D, D)], dst, sems.at[XC + part])

    def w_copy(j):
        src, dst = [(w1_hbm, w1_v), (wo_hbm, wo_v), (w2_hbm, w2_v), (w3_hbm, w3_v), (w4_hbm, w4_v)][j]
        return pltpu.make_async_copy(src, dst, sems.at[XC + 3 + j])

    @pl.when(i == 0)
    def _prologue():
        wqkv_copy(1).start()
        x_copy(0).start()
        x_copy(1).start()
        w_copy(0).start()
        wqkv_copy(0).start()
        wqkv_copy(2).start()
        x_copy(2).start()
        x_copy(3).start()
        for j in range(1, 5):
            w_copy(j).start()

        grp = (jax.lax.broadcasted_iota(jnp.int32, (H, D), 1) // DH
               == jax.lax.broadcasted_iota(jnp.int32, (H, D), 0)).astype(_bf)

        def k_proj(c):
            kb = jnp.dot(x_v[c * XR:(c + 1) * XR, :], wk_v[...],
                         preferred_element_type=_f32).astype(_bf)
            k_scr[c * XR // 2:(c + 1) * XR // 2, :] = _pack(kb)
            kf = kb.astype(_f32)
            return (kf * kf).astype(_bf)

        def k_norm2(k2):
            n2 = jax.lax.dot_general(grp, k2, _NT, preferred_element_type=_f32)
            return jnp.max(n2.reshape(H, XR // 128, 128), axis=1)

        def ln_x(c):
            return _layernorm(x_v[c * XR:(c + 1) * XR, :].astype(_f32)).astype(_bf)

        def h_proj(c, ln):
            hh = _gelu(jnp.dot(ln, w1_v[...], preferred_element_type=_f32))
            h_scr[PAD + c * XR:PAD + (c + 1) * XR, :] = hh.astype(_bf).astype(_f32)

        h_scr[0:PAD, :] = jnp.zeros((PAD, D), _f32)
        h_scr[PAD + S:PAD + S + PAD, :] = jnp.zeros((PAD, D), _f32)
        for sl in range(NSLOT - LA, NSLOT):
            p_scr[sl] = jnp.zeros((KC, TQ), _bf)

        wqkv_copy(1).wait()
        x_copy(0).wait()
        k2_0 = k_proj(0)
        ln_0 = ln_x(0)
        x_copy(1).wait()
        w_copy(0).wait()
        k2_1 = k_proj(1)
        ln_1 = ln_x(1)
        h_proj(0, ln_0)
        kn2 = k_norm2(k2_0)
        h_proj(1, ln_1)
        kn2 = jnp.maximum(kn2, k_norm2(k2_1))
        wqkv_copy(0).wait()
        wqkv_copy(2).wait()
        x_copy(2).wait()
        x_copy(3).wait()
        wq_t = wq_v[...].astype(_f32).T.astype(_bf)
        wv_t = wv_v[...].astype(_f32).T.astype(_bf)
        k2_2 = k_proj(2)
        ln_2 = ln_x(2)
        k2_3 = k_proj(3)
        ln_3 = ln_x(3)
        h_proj(2, ln_2)
        kn2 = jnp.maximum(kn2, k_norm2(k2_2))
        h_proj(3, ln_3)
        kn2 = jnp.maximum(kn2, k_norm2(k2_3))
        kn2 = jnp.max(kn2, axis=1, keepdims=True)
        xa = x_v[...]
        qt = jax.lax.dot_general(wq_t, xa, _NT, preferred_element_type=_f32)
        qtb = (qt * (DH ** -0.5 * LOG2E)).astype(_bf)
        qt_scr[...] = qtb
        vt_scr[...] = _pack(
            jax.lax.dot_general(wv_t, xa, _NT, preferred_element_type=_f32).astype(_bf))
        qf = qtb.astype(_f32)
        qn2 = jnp.sum((qf * qf).reshape(H, DH, S), axis=1)
        m_scr[...] = jnp.sqrt(qn2 * kn2) * 1.02
        for j in range(1, 5):
            w_copy(j).wait()

    q0 = pl.multiple_of(i * TQ, TQ)
    rows = jax.lax.broadcasted_iota(jnp.int32, (128, TQ), 0) // DH

    def masked_q(h):
        goff = pl.multiple_of((h // 8) * 128, 128)
        qg = qt_scr[pl.ds(goff, 128), pl.ds(q0, TQ)]
        return jnp.where(rows == (h % 8), qg, jnp.zeros_like(qg)), goff

    def pv_dot(h, kc, sl):
        vt = _unpack(vt_scr[pl.ds(pl.multiple_of(h * (DH // 2), DH // 2), DH // 2),
                            kc * KC:(kc + 1) * KC])
        return jnp.dot(vt, p_scr[sl], preferred_element_type=_f32)

    def store_acc(h, acc):
        acc_scr[pl.ds(pl.multiple_of((h + 1) * DH, DH), DH), :] = acc

    NW = HPI * NC
    tail = [(NC - LA + t, (NW - LA + t) % NSLOT) for t in range(LA)]

    def fast_heads(g, acc_prev):
        h0 = g * HPI
        qms = [masked_q(h0 + u)[0] for u in range(HPI)]
        goff = masked_q(h0)[1]
        ms = [m_scr[pl.ds(h0 + u, 1), pl.ds(q0, TQ)] for u in range(HPI)]
        work = [(u, kc) for u in range(HPI) for kc in range(NC)]
        accs = [jnp.zeros((DH, TQ), _f32) for _ in range(HPI)]
        ls = [jnp.zeros((8, TQ), _f32) for _ in range(HPI)]

        hprev = jnp.maximum(h0 - 1, 0)
        for kc, sl in tail:
            acc_prev = acc_prev + pv_dot(hprev, kc, sl)
        store_acc(h0 - 1, acc_prev)

        def qk_step(idx):
            u, kc = work[idx]
            kc_val = _unpack(k_scr[kc * KC // 2:(kc + 1) * KC // 2, pl.ds(goff, 128)])
            s = jnp.dot(kc_val, qms[u], preferred_element_type=_f32)
            p32 = jnp.exp2(s - ms[u])
            ls[u] = ls[u] + jnp.sum(p32.reshape(KC // 8, 8, TQ), axis=0)
            p_scr[idx % NSLOT] = p32.astype(_bf)
            if kc == NC - 1:
                l_scr[h0 + u] = ls[u]

        def pv_step(idx):
            u, kc = work[idx]
            accs[u] = accs[u] + pv_dot(h0 + u, kc, idx % NSLOT)
            if kc == NC - 1:
                store_acc(h0 + u, accs[u])

        for idx in range(NW - LA):
            qk_step(idx)
            if idx >= LA:
                pv_step(idx - LA)
        for idx in range(NW - LA, NW):
            qk_step(idx)
        for idx in range(NW - 2 * LA, NW - LA):
            pv_step(idx)
        return accs[HPI - 1]

    acc_last = jax.lax.fori_loop(0, H // HPI, fast_heads, jnp.zeros((DH, TQ), _f32))
    for kc, sl in tail:
        acc_last = acc_last + pv_dot(H - 1, kc, sl)
    store_acc(H - 1, acc_last)

    c = D // 4
    win = h_scr[pl.ds(q0, TQ + 2 * PAD), :]
    hs_in = jnp.concatenate([
        win[PAD - 1:PAD - 1 + TQ, 0 * c:1 * c],
        win[PAD + 1:PAD + 1 + TQ, 1 * c:2 * c],
        win[PAD - 2:PAD - 2 + TQ, 2 * c:3 * c],
        win[PAD + 2:PAD + 2 + TQ, 3 * c:4 * c]], axis=-1).astype(_bf)
    xa_t = x_v[pl.ds(q0, TQ), :].astype(_f32)
    x1 = xa_t + jnp.dot(hs_in, w2_v[...], preferred_element_type=_f32)

    def attn_out():
        l_all = jnp.sum(l_scr[...], axis=1)
        ot = acc_scr[DH:, :].reshape(H, DH, TQ) * (1.0 / l_all)[:, None, :]
        ot = ot.reshape(D, TQ).astype(_bf)
        return jax.lax.dot_general(ot, wo_v[...], _TN, preferred_element_type=_f32), l_all

    a, l_all = attn_out()
    safe = jnp.logical_and(jnp.min(l_all) >= 2.0 ** -79, jnp.max(l_all) <= 2.0 ** 100)

    h3 = _gelu(jnp.dot(_layernorm(x1).astype(_bf), w3_v[...], preferred_element_type=_f32))
    b = x1 + jnp.dot(h3.astype(_bf), w4_v[...], preferred_element_type=_f32)
    g = jax.nn.sigmoid(jnp.sum(xa_t * gw_ref[...].astype(_f32).reshape(1, D), axis=-1, keepdims=True))
    gb = (1.0 - g) * b
    gb_scr[...] = gb
    o_ref[...] = (g * a + gb).astype(o_ref.dtype)

    @pl.when(jnp.logical_not(safe))
    def _fallback():
        def slow_head(t, carry):
            h = t // (TQ // 128)
            q1 = pl.multiple_of((t % (TQ // 128)) * 128, 128)
            goff = pl.multiple_of((h // 8) * 128, 128)
            qg = qt_scr[pl.ds(goff, 128), pl.ds(q0 + q1, 128)]
            qm = jnp.where(rows[:, :128] == (h % 8), qg, jnp.zeros_like(qg))
            s = jnp.dot(_unpack(k_scr[:, pl.ds(goff, 128)]), qm, preferred_element_type=_f32)
            p32 = jnp.exp2(s - jnp.max(s, axis=0, keepdims=True))
            l_scr[h, :, pl.ds(q1, 128)] = jnp.sum(p32.reshape(S // 8, 8, 128), axis=0)
            vt = _unpack(vt_scr[pl.ds(pl.multiple_of(h * (DH // 2), DH // 2), DH // 2), :])
            acc_scr[pl.ds(pl.multiple_of((h + 1) * DH, DH), DH), pl.ds(q1, 128)] = jnp.dot(
                vt, p32.astype(_bf), preferred_element_type=_f32)
            return carry
        jax.lax.fori_loop(0, H * (TQ // 128), slow_head, 0)
        a2, _ = attn_out()
        g2 = jax.nn.sigmoid(jnp.sum(x_v[pl.ds(q0, TQ), :].astype(_f32) * gw_ref[...].astype(_f32).reshape(1, D),
                                    axis=-1, keepdims=True))
        o_ref[...] = (g2 * a2 + gb_scr[...]).astype(o_ref.dtype)


@jax.jit
def pallas_gated_mix__mha_block__mixer_s_mlp__prompt_kernel(
    A_x: jax.Array,
    A_wqkv: jax.Array,
    A_wo: jax.Array,
    B_x: jax.Array,
    B_w1: jax.Array,
    B_w2: jax.Array,
    B_w3: jax.Array,
    B_w4: jax.Array,
    gate_w: jax.Array,
):
    hbm = pl.BlockSpec(memory_space=pl.ANY)
    out = pl.pallas_call(
        _kernel,
        grid=(S // TQ,),
        in_specs=[hbm] * 7 + [pl.BlockSpec((D,), lambda i: (0,))],
        out_specs=pl.BlockSpec((TQ, D), lambda i: (i, 0)),
        out_shape=jax.ShapeDtypeStruct((S, D), jnp.bfloat16),
        scratch_shapes=[
            pltpu.VMEM((S, D), _bf),
            pltpu.VMEM((D, D), _bf),
            pltpu.VMEM((D, D), _bf),
            pltpu.VMEM((D, D), _bf),
            pltpu.VMEM((D, D), _bf),
            pltpu.VMEM((D, D), _bf),
            pltpu.VMEM((D, D), _bf),
            pltpu.VMEM((D, F), _bf),
            pltpu.VMEM((F, D), _bf),
            pltpu.SemaphoreType.DMA((XC + 3 + 5,)),
            pltpu.VMEM((S // 2, D), jnp.uint32),
            pltpu.VMEM((D, S), _bf),
            pltpu.VMEM((D // 2, S), jnp.uint32),
            pltpu.VMEM((H, S), _f32),
            pltpu.VMEM((S + 2 * PAD, D), _f32),
            pltpu.VMEM(((H + 1) * DH, TQ), _f32),
            pltpu.VMEM((H, 8, TQ), _f32),
            pltpu.VMEM((NSLOT, KC, TQ), _bf),
            pltpu.VMEM((TQ, D), _f32),
        ],
        compiler_params=pltpu.CompilerParams(
            dimension_semantics=("arbitrary",),
            vmem_limit_bytes=100 * 1024 * 1024),
        name="gated_mix",
    )(A_x.reshape(S, D), A_wqkv, A_wo, B_w1, B_w2, B_w3, B_w4, gate_w)
    return out.reshape(1, S, D)
```
